```python
import os as _os
_os.environ.setdefault("JAX_PLATFORMS", "cpu")
import jax
import jax.numpy as jnp

def _softmax(x, axis=-1):
    return jax.nn.softmax(x, axis=axis)
def _gelu(x):
    return jax.nn.gelu(x, approximate=True)
def _silu(x):
    return jax.nn.silu(x)
def _sigmoid(x):
    return jax.nn.sigmoid(x)
def _layernorm(x, axis=-1, eps=1e-5):
    m = jnp.mean(x, axis=axis, keepdims=True)
    v = jnp.var(x, axis=axis, keepdims=True)
    return (x - m) / jnp.sqrt(v + eps)
def _scatter_add(tgt, idx, src, axis=0):
    return tgt.at[idx].add(src)
def _segment_sum(src, seg, n):
    return jax.ops.segment_sum(src, seg, n)
class _Rng:
    def __init__(self, key):
        self._k = key
    def _next(self):
        self._k, sub = jax.random.split(self._k)
        return sub
    def normal(self, shape):
        return jax.random.normal(self._next(), shape, dtype=jnp.bfloat16)
    def randint(self, lo, hi, shape):
        return jax.random.randint(self._next(), shape, lo, hi, dtype=jnp.int32)
    def uniform(self, shape, lo=0.0, hi=1.0):
        return jax.random.uniform(self._next(), shape, jnp.bfloat16, lo, hi)
    def permutation(self, n):
        return jax.random.permutation(self._next(), n)


kernel_name = 'parallel_sum__grouped_kv_mqa__dense_activation_silu__prompt'

def setup_inputs():
    _rng = _Rng(jax.random.key(int.from_bytes(__import__("os").urandom(4), "little")))
    _w = (lambda a: (lambda t: t.astype(jnp.bfloat16) if jnp.issubdtype(t.dtype, jnp.floating) else t)(jnp.asarray(a)))
    def _A_setup():
        B, S, D, H = 1, 2048, 512, 32
        Dh = D // H
        return {
            "x": _w((lambda *s: _rng.normal(s) * 0.05)(B, S, D)),
            "wq": _w((lambda *s: _rng.normal(s) * 0.05)(D, H * Dh)),
            "wk": _w((lambda *s: _rng.normal(s) * 0.05)(D, Dh)),
            "wv": _w((lambda *s: _rng.normal(s) * 0.05)(D, Dh)),
            "wo": _w((lambda *s: _rng.normal(s) * 0.05)(H * Dh, D)),
        }
    _A_in = _A_setup()

    def _B_setup():
        B, S, D, F = 1, 2048, 512, 1792
        return {
            "x": _w((lambda *s: _rng.normal(s) * 0.05)(B, S, D)),
            "w1": _w((lambda *s: _rng.normal(s) * 0.05)(D, F) * (D ** -0.5)),
            "w2": _w((lambda *s: _rng.normal(s) * 0.05)(F, D) * (F ** -0.5)),
        }
    _B_in = _B_setup()

    return {
        "A_x": _A_in["x"],
        "A_wq": _A_in["wq"],
        "A_wk": _A_in["wk"],
        "A_wv": _A_in["wv"],
        "A_wo": _A_in["wo"],
        "B_x": _B_in["x"],
        "B_w1": _B_in["w1"],
        "B_w2": _B_in["w2"],
    }

def reference(A_x, A_wq, A_wk, A_wv, A_wo, B_x, B_w1, B_w2):
    def _A_ref(x, wq, wk, wv, wo):
        B, S, D = x.shape
        H = 32
        Dh = D // H
        q = (lambda x, *d: x.transpose(*d))((x @ wq).reshape(B, S, H, Dh), 0, 2, 1, 3)
        k = x @ wk
        v = x @ wv
        scores = jnp.einsum("bhqd,bkd->bhqk", q, k) * (Dh ** -0.5)
        p = _softmax(scores, axis=-1)
        o = jnp.einsum("bhqk,bkd->bhqd", p, v)
        return (lambda x, *d: x.transpose(*d))(o, 0, 2, 1, 3).reshape(B, S, H * Dh) @ wo

    def _B_ref(x, w1, w2):
        h = jnp.einsum("bsd,df->bsf", x, w1)
        h = _silu(h)
        out = jnp.einsum("bsf,fd->bsd", h, w2)
        return out

    x = A_x
    xn = _layernorm(x, axis=-1)
    return x + _A_ref(xn, A_wq, A_wk, A_wv, A_wo) + _B_ref(xn, B_w1, B_w2)
```

```python
import functools
import jax
import jax.numpy as jnp
from jax import lax
import jax.experimental.pallas as pl
import jax.experimental.pallas.tpu as pltpu

S, D, H, DH, F = 2048, 512, 32, 16, 1792
CD = 32
LOG2E = 1.4426950408889634
EPS = 1e-5
NT_DIMS = (((1,), (1,)), ((), ()))
L_LO, L_HI = 2.0 ** -40, 2.0 ** 40


def make_kernel(TQ=512, KC=128, LAG=2, HPI=8, KV=16, UW=128, NX=8, tree=1, fallback=True):
    NC = S // KC
    KM = KC - KV
    NU = TQ // UW
    f32, bf16 = jnp.float32, jnp.bfloat16
    RB = S // NX

    def kernel(x_hbm, wq_hbm, wk_hbm, wv_hbm, wo_hbm, w1_hbm, w2_hbm, o_ref,
               x_s, wq_s, wk_s, wv_s, wo_s, w1_s, w2_s, sems,
               xn_s, wqT_s, wkv_s, k_s, vT_s, kb_s, kmax_s, qT_s, qf_s, qb_s, oT_s):
        i = pl.program_id(0)
        x_cp = [pltpu.make_async_copy(x_hbm.at[pl.ds(r * RB, RB)], x_s.at[pl.ds(r * RB, RB)], sems.at[r])
                for r in range(NX)]
        w_cp = [pltpu.make_async_copy(src, dst, sems.at[NX + n]) for n, (src, dst) in enumerate(
            [(wk_hbm, wk_s), (wv_hbm, wv_s), (wq_hbm, wq_s), (wo_hbm, wo_s), (w1_hbm, w1_s), (w2_hbm, w2_s)])]

        @pl.when(i == 0)
        def _prologue():
            x_cp[0].start()
            for cp in w_cp[:3]: cp.start()
            for cp in x_cp[1:]: cp.start()
            for cp in w_cp[3:]: cp.start()
            for r in range(NX):
                x_cp[r].wait()
                rows = pl.ds(r * RB, RB)
                x = x_s[rows, :].astype(f32)
                m = jnp.mean(x, axis=-1, keepdims=True)
                xc = x - m
                v = jnp.mean(xc * xc, axis=-1, keepdims=True)
                xn_s[rows, :] = (xc * lax.rsqrt(v + EPS)).astype(bf16)
            for cp in w_cp[:3]: cp.wait()
            wqT_s[...] = wq_s[...].astype(f32).T.astype(bf16)
            wkv_s[...] = jnp.zeros(wkv_s.shape, f32)
            wkv_s[:, 0:DH] = wk_s[...].astype(f32)
            wkv_s[:, DH:2 * DH] = wv_s[...].astype(f32)
            wkvT = wkv_s[...].T[0:2 * DH, :].astype(bf16)
            kvT = lax.dot_general(wkvT, xn_s[...], NT_DIMS, preferred_element_type=f32)
            vT_s[...] = kvT[DH:2 * DH, :].astype(bf16)
            kT = kvT[0:DH, :].astype(bf16).astype(f32)
            kn2 = jnp.sum(kT * kT, axis=0, keepdims=True)
            kmax = jnp.sqrt(jnp.max(kn2, axis=1, keepdims=True))
            kmax_s[...] = jnp.broadcast_to(kmax, kmax_s.shape)
            sub = lax.broadcasted_iota(jnp.int32, (128 - DH, S), 0)
            kfull = jnp.concatenate([kT, jnp.where(sub == 0, 1.0, 0.0)], axis=0).T
            k_s[...] = kfull.astype(bf16)
            if KV:
                kv_rows = kfull.reshape(NC, KC, 128)[:, KM:, :].reshape(NC * KV, 128)
                for d in range(DH):
                    kb_s[d] = jnp.broadcast_to(kv_rows[:, d:d + 1], (NC * KV, 128))

        rows = pl.ds(pl.multiple_of(i * TQ, TQ), TQ)
        qT = lax.dot_general(wqT_s[...], xn_s[rows, :], NT_DIMS, preferred_element_type=f32) * (DH ** -0.5 * LOG2E)
        q3 = qT.reshape(H, DH, TQ)
        qn = jnp.sqrt(jnp.sum(q3 * q3, axis=1, keepdims=True))
        kmax = jnp.tile(kmax_s[0:1, :], (1, TQ // 128))
        shift = -(qn * kmax * (1.0 + 2.0 ** -6))
        sub = lax.broadcasted_iota(jnp.int32, (H, DH, TQ), 1)
        extra = jnp.where(sub == 0, jnp.broadcast_to(shift, (H, DH, TQ)), 0.0)
        qb = jnp.concatenate([q3, extra], axis=1).astype(bf16)
        qT_s[...] = qb
        if KV:
            qf_s[...] = qb[:, 0:24, :].astype(f32)

        def heads(hh, ok):
            seq = [(j, c) for j in range(HPI) for c in range(NC)]
            accs = [jnp.zeros((DH, TQ), f32) for _ in range(HPI)]
            ls = [[jnp.zeros((8, UW), f32) for _ in range(NU)] for _ in range(HPI)]
            ps, pvs, qrows = {}, {}, {}

            def stage_q(j):
                for d in range(DH + 1):
                    qb_s[j, d * 8:(d + 1) * 8, :] = jnp.broadcast_to(qf_s[hh * HPI + j, d:d + 1, :], (8, TQ))

            def get_q(j, d, u):
                return jnp.tile(qb_s[j, d * 8:(d + 1) * 8, u * UW:(u + 1) * UW], (KV // 8, 1))

            def unit(n, u):
                j, c = seq[n]
                terms = [get_q(j, DH, u)] + [None] * (tree - 1)
                for d in range(DH):
                    t = jnp.tile(kb_s[d, c * KV:(c + 1) * KV, :], (1, UW // 128)) * get_q(j, d, u)
                    a = d % tree
                    terms[a] = t if terms[a] is None else terms[a] + t
                sv = functools.reduce(lambda a, b: a + b, terms)
                p = jnp.exp2(sv)
                for r in range(KV // 8):
                    ls[j][u] = ls[j][u] + p[r * 8:(r + 1) * 8]
                pvs[(n, u)] = p

            def qk(n):
                j, c = seq[n]
                NR = KM // 8
                where = {((2 * u + 1) * NR) // (2 * NU): u for u in range(NU)} if KV else {}
                s = jnp.dot(k_s[c * KC:c * KC + KM, 0:CD], qT_s[hh * HPI + j], preferred_element_type=f32)
                p = jnp.exp2(s)
                for r in range(NR):
                    for u in range(NU):
                        ls[j][u] = ls[j][u] + p[r * 8:(r + 1) * 8, u * UW:(u + 1) * UW]
                    if r in where:
                        unit(n, where[r])
                ps[n] = p

            def pv(n):
                j, c = seq[n]
                p = ps.pop(n)
                if KV:
                    p = jnp.concatenate([p, jnp.concatenate([pvs.pop((n, u)) for u in range(NU)], axis=1)], axis=0)
                accs[j] = accs[j] + jnp.dot(vT_s[:, c * KC:(c + 1) * KC], p.astype(bf16), preferred_element_type=f32)

            n = len(seq)
            if KV: stage_q(0)
            for t in range(n + LAG):
                if KV and t % NC == NC // 2 and t // NC + 1 < HPI: stage_q(t // NC + 1)
                if t < n: qk(t)
                if t - LAG >= 0: pv(t - LAG)
            for j in range(HPI):
                l = jnp.sum(jnp.concatenate(ls[j], axis=1), axis=0, keepdims=True)
                ok = jnp.minimum(ok, jnp.where((l >= L_LO) & (l <= L_HI), 1.0, 0.0))
                oT_s[pl.ds(pl.multiple_of((hh * HPI + j) * DH, DH), DH), :] = accs[j] / l
            return ok
        ok = lax.fori_loop(0, H // HPI, heads, jnp.ones((1, TQ), f32))

        if fallback:
            @pl.when(jnp.min(ok) < 0.5)
            def _true_max_softmax():
                KB = 256
                def head(h, _):
                    q = qT_s[h, 0:DH, :]
                    def chunk(c, carry):
                        m, l, acc = carry
                        ks = pl.ds(pl.multiple_of(c * KB, KB), KB)
                        s = jnp.dot(k_s[ks, 0:DH], q, preferred_element_type=f32)
                        m_new = jnp.maximum(m, jnp.max(s, axis=0, keepdims=True))
                        alpha = jnp.exp2(m - m_new)
                        p = jnp.exp2(s - m_new)
                        l = l * alpha + jnp.sum(p, axis=0, keepdims=True)
                        acc = acc * alpha + jnp.dot(vT_s[:, ks], p.astype(bf16), preferred_element_type=f32)
                        return m_new, l, acc
                    m, l, acc = lax.fori_loop(0, S // KB, chunk, (
                        jnp.full((1, TQ), -jnp.inf, f32), jnp.zeros((1, TQ), f32), jnp.zeros((DH, TQ), f32)))
                    oT_s[pl.ds(pl.multiple_of(h * DH, DH), DH), :] = acc / l
                    return 0
                lax.fori_loop(0, H, head, 0)

        @pl.when(i == 0)
        def _():
            for cp in w_cp[3:]: cp.wait()

        o = oT_s[...].T.astype(bf16)
        a = jnp.dot(o, wo_s[...], preferred_element_type=f32)
        h = jnp.dot(xn_s[rows, :], w1_s[...], preferred_element_type=f32)
        h = h * jax.nn.sigmoid(h)
        b = jnp.dot(h.astype(bf16), w2_s[...], preferred_element_type=f32)
        o_ref[...] = (x_s[rows, :].astype(f32) + a + b).astype(o_ref.dtype)

    @jax.jit
    def run(A_x, A_wq, A_wk, A_wv, A_wo, B_x, B_w1, B_w2):
        x = A_x.reshape(S, D)
        out = pl.pallas_call(
            kernel,
            grid=(S // TQ,),
            in_specs=[pl.BlockSpec(memory_space=pl.ANY)] * 7,
            out_specs=pl.BlockSpec((TQ, D), lambda i: (i, 0)),
            out_shape=jax.ShapeDtypeStruct((S, D), A_x.dtype),
            scratch_shapes=[
                pltpu.VMEM((S, D), bf16), pltpu.VMEM((D, D), bf16), pltpu.VMEM((D, DH), bf16),
                pltpu.VMEM((D, DH), bf16), pltpu.VMEM((D, D), bf16), pltpu.VMEM((D, F), bf16),
                pltpu.VMEM((F, D), bf16), pltpu.SemaphoreType.DMA((NX + 6,)),
                pltpu.VMEM((S, D), bf16),
                pltpu.VMEM((D, D), bf16),
                pltpu.VMEM((D, 128), f32),
                pltpu.VMEM((S, 128), bf16),
                pltpu.VMEM((DH, S), bf16),
                pltpu.VMEM((DH, max(NC * KV, 8), 128), f32),
                pltpu.VMEM((8, 128), f32),
                pltpu.VMEM((H, CD, TQ), bf16),
                pltpu.VMEM((H, 24, TQ), f32),
                pltpu.VMEM((HPI, (DH + 1) * 8, TQ), f32),
                pltpu.VMEM((D, TQ), f32),
            ],
            compiler_params=pltpu.CompilerParams(
                dimension_semantics=("arbitrary",), vmem_limit_bytes=100 * 2 ** 20),
        )(x, A_wq, A_wk, A_wv, A_wo, B_w1, B_w2)
        return out.reshape(A_x.shape)
    return run


pallas_parallel_sum__grouped_kv_mqa__dense_activation_silu__prompt_kernel = make_kernel(HPI=8)
```

```python
import functools
import jax
import jax.numpy as jnp
from jax import lax
import jax.experimental.pallas as pl
import jax.experimental.pallas.tpu as pltpu

S, D, H, DH, F = 2048, 512, 32, 16, 1792
LOG2E = 1.4426950408889634
EPS = 1e-5
NT_DIMS = (((1,), (1,)), ((), ()))
L_LO, L_HI = 2.0 ** -40, 2.0 ** 40
TQ, KC, UW, KV = 512, 128, 128, 16
KM = KC - KV
NC, NU, NT, NF = S // KC, TQ // UW, S // TQ, F // 128
CPT = TQ // KC


def make_kernel(LAG=2, HPI=8, fallback=True, scopes=False, NVT=3, bounds=(0, 8, 16, 24), dl=(9, 17, 25)):
    anchor = 1
    NI = H // HPI
    FR = TQ // NI
    GW = HPI * DH
    f32, bf16 = jnp.float32, jnp.bfloat16
    scope = jax.named_scope if scopes else (lambda name: (lambda f: f))

    def kernel(x_hbm, wq_hbm, wkT_hbm, wvT_hbm, wo_hbm, w1_hbm, w2_hbm, o_ref,
               x_s, wq_s, wo_s, w1_s, w2_s, sems,
               xn_s, wT_s, k_s, vT_s, kb_s, kb2_s, zero_s, qT_s, qf_s, sh_s, oh_s, y_s):
        i = pl.program_id(0)
        x_cp = [pltpu.make_async_copy(x_hbm.at[pl.ds(t * TQ, TQ)], x_s.at[pl.ds(t * TQ, TQ)], sems.at[t])
                for t in range(NT)]
        w_cp = [pltpu.make_async_copy(src, dst, sems.at[NT + n]) for n, (src, dst) in enumerate(
            [(wq_hbm, wq_s), (wkT_hbm, wT_s.at[pl.ds(0, DH)]), (wvT_hbm, wT_s.at[pl.ds(DH, DH)]),
             (w1_hbm, w1_s), (w2_hbm, w2_s), (wo_hbm, wo_s)])]

        @pl.when(i == 0)
        @scope("prologue")
        def _prologue():
            x_cp[0].start()
            for cp in w_cp[:3]: cp.start()
            for cp in x_cp[1:]: cp.start()
            for cp in w_cp[3:]: cp.start()
            zero_s[...] = jnp.zeros(zero_s.shape, f32)

            def ln(t):
                rows = pl.ds(t * TQ, TQ)
                x = x_s[rows, :].astype(f32)
                m = jnp.mean(x, axis=-1, keepdims=True)
                xc = x - m
                v = jnp.mean(xc * xc, axis=-1, keepdims=True)
                xn_s[rows, :] = (xc * lax.rsqrt(v + EPS)).astype(bf16)

            hrow = lax.broadcasted_iota(jnp.int32, (H, D), 0)
            hcol = lax.broadcasted_iota(jnp.int32, (H, D), 1)
            blockdiag = jnp.where(hcol // DH == hrow, 1.0, 0.0).astype(bf16)

            def proj(t):
                rows = pl.ds(t * TQ, TQ)
                res = lax.dot_general(wT_s[...], xn_s[rows, :], NT_DIMS, preferred_element_type=f32)
                qb = (res[2 * DH:] * (DH ** -0.5 * LOG2E)).astype(bf16)
                qT_s[t * H:(t + 1) * H] = qb.reshape(H, DH, TQ)
                qf = qb.astype(f32)
                qf_s[t * H:(t + 1) * H] = qf.reshape(H, DH, TQ)
                qn2 = jnp.dot(blockdiag, (qf * qf).astype(bf16), preferred_element_type=f32)
                vT_s[:, rows] = res[DH:2 * DH].astype(bf16)
                kT = res[0:DH].astype(bf16).astype(f32)
                sub = lax.broadcasted_iota(jnp.int32, (128 - DH, TQ), 0)
                kfull = jnp.concatenate([kT, jnp.where(sub == 0, 1.0, 0.0)], axis=0).T
                k_s[rows, :] = kfull.astype(bf16)
                kv_rows = kfull.reshape(CPT, KC, 128)[:, KM:, :].reshape(CPT * KV, 128)
                for d in range(DH):
                    kb_s[d, t * CPT * KV:(t + 1) * CPT * KV, :] = jnp.broadcast_to(kv_rows[:, d:d + 1], (CPT * KV, 128))
                if t == NT - 1 and NVT:
                    for d in range(DH):
                        kb2_s[d] = jnp.broadcast_to(kfull[TQ - KC:, d:d + 1], (KC, 128))
                return jnp.sqrt(qn2), jnp.sum(kT * kT, axis=0, keepdims=True)

            x_cp[0].wait()
            ln(0)
            for cp in w_cp[:3]: cp.wait()
            wT_s[2 * DH:, :] = wq_s[...].astype(f32).T.astype(bf16)
            st = [proj(0)]
            for cp in x_cp[1:]: cp.wait()
            ln(1)
            st.append(proj(1))
            ln(2)
            st.append(proj(2))
            ln(3)
            st.append(proj(3))
            kn2 = functools.reduce(jnp.maximum, [s[1] for s in st])
            nkmax = jnp.sqrt(jnp.max(kn2, axis=1, keepdims=True)) * -(1.0 + 2.0 ** -6)
            for t in range(NT):
                sh_s[t * NI:(t + 1) * NI] = (st[t][0] * nkmax).astype(bf16).astype(f32).reshape(NI, HPI, TQ)
            for cp in w_cp[3:5]: cp.wait()

        def heads(hh, ok):
            h0 = i * H + hh * HPI
            frows = pl.ds(pl.multiple_of(i * TQ + hh * FR, FR), FR)
            n = HPI * NC
            accs = [zero_s[0:DH, :] for _ in range(HPI)]
            ls = [[jnp.zeros((8, UW), f32) for _ in range(NU)] for _ in range(HPI)]
            ps, pvs, hact, wts = {}, {}, {}, {}
            y = [None] * 4
            row0 = lax.broadcasted_iota(jnp.int32, (DH, UW), 0) == 0

            def shift(j, u):
                return jnp.broadcast_to(sh_s[i * NI + hh, j:j + 1, u * UW:(u + 1) * UW], (KV, UW))

            def weights(j):
                if j not in wts:
                    extra = jnp.concatenate([jnp.where(row0, shift(j, u), 0.0) for u in range(NU)], axis=1)
                    wts[j] = jnp.concatenate([qT_s[h0 + j], extra.astype(bf16)], axis=0)
                return wts[j]

            def unit(t, u):
                j, c = divmod(t, NC)
                sv = shift(j, u)
                for d in range(DH):
                    qd = jnp.broadcast_to(qf_s[h0 + j, d:d + 1, u * UW:(u + 1) * UW], (KV, UW))
                    sv = sv + kb_s[d, c * KV:(c + 1) * KV, :] * qd
                p = jnp.exp2(sv)
                ls[j][u] = ls[j][u] + p[0:8] + p[8:16]
                pvs[(t, u)] = p

            def qk(t):
                j, c = divmod(t, NC)
                NR = KM // 8
                where = {((2 * u + 1) * NR) // (2 * NU): u for u in range(NU)}
                s = jnp.dot(k_s[c * KC:c * KC + KM, 0:2 * DH], weights(j), preferred_element_type=f32)
                p = jnp.exp2(s)
                for r in range(NR):
                    for u in range(NU):
                        ls[j][u] = ls[j][u] + p[r * 8:(r + 1) * 8, u * UW:(u + 1) * UW]
                    if r in where:
                        unit(t, where[r])
                ps[t] = p

            def pv(t):
                j, c = divmod(t, NC)
                p = jnp.concatenate([ps.pop(t), jnp.concatenate([pvs.pop((t, u)) for u in range(NU)], axis=1)], axis=0)
                accs[j] = accs[j] + jnp.dot(vT_s[:, c * KC:(c + 1) * KC], p.astype(bf16), preferred_element_type=f32)

            def w1(m0, m1):
                hm = 0.5 * jnp.dot(xn_s[frows, :], w1_s[:, m0 * 128:m1 * 128], preferred_element_type=f32)
                return (hm + hm * jnp.tanh(hm)).astype(bf16)

            vheads = list(range(HPI - NVT, HPI))
            order = [t for t in range(n) if not (t % NC == NC - 1 and t // NC in vheads)]
            always = zero_s[0:8, 0:UW] == 0.0

            def vunit(j, g, u, anc):
                if anc is not None:
                    ls[j][u] = jnp.where(always, ls[j][u], anc)
                sv = shift(j, u)
                for d in range(DH):
                    qd = jnp.broadcast_to(qf_s[h0 + j, d:d + 1, u * UW:(u + 1) * UW], (KV, UW))
                    sv = sv + kb2_s[d, g * KV:(g + 1) * KV, :] * qd
                p = jnp.exp2(sv)
                ls[j][u] = ls[j][u] + p[0:8] + p[8:16]
                pvs[('v', j, g, u)] = p

            def vpv(j):
                p = jnp.concatenate([jnp.concatenate([pvs.pop(('v', j, g, u)) for u in range(NU)], axis=1)
                                     for g in range(KC // KV)], axis=0)
                accs[j] = accs[j] + jnp.dot(vT_s[:, S - KC:], p.astype(bf16), preferred_element_type=f32)

            w2p = [[('w2', (4 * g, 4 * g + 4, nn, nn + 1)) for nn in range(4)] for g in range(3)]
            w2p.append([('w2', (12, 14, 0, 2)), ('w2', (12, 14, 2, 4))])
            w1p = [('w1', m) for m in range(NF)]
            pieces = w1p[0:5]
            for k in range(4): pieces += [w2p[0][k], w1p[5 + k]]
            for k in range(4): pieces += [w2p[1][k], w1p[9 + k]]
            pieces += [w2p[2][0], w1p[13]] + w2p[2][1:] + w2p[3]
            where2 = {}
            for sidx, j in enumerate(vheads):
                rows_ = [divmod(q, 16) for q in range(int(bounds[sidx] * 16), int(bounds[sidx + 1] * 16))]
                us = [(j, g, u) for g in range(KC // KV) for u in range(NU)]
                for k, un in enumerate(us):
                    where2[rows_[((2 * k + 1) * len(rows_)) // (2 * len(us))]] = un

            def piece(k):
                kind, a = pieces[k]
                if kind == 'w1':
                    res = jnp.dot(xn_s[frows, :], w1_s[:, a * 128:(a + 1) * 128], preferred_element_type=f32)
                else:
                    k0, k1, n0, n1 = a
                    res = jnp.dot(jnp.concatenate([hact[kk] for kk in range(k0, k1)], axis=1),
                                  w2_s[k0 * 128:k1 * 128, n0 * 128:n1 * 128], preferred_element_type=f32)
                for r in range(16):
                    if (k, r) in where2:
                        vunit(*where2[(k, r)], res[r * 8:(r + 1) * 8, 0:UW] if anchor else None)
                if kind == 'w1':
                    hm = 0.5 * res
                    hact[a] = (hm + hm * jnp.tanh(hm)).astype(bf16)
                else:
                    for nn in range(n0, n1):
                        pn = res[:, (nn - n0) * 128:(nn - n0 + 1) * 128]
                        y[nn] = pn if y[nn] is None else y[nn] + pn

            for k, t in enumerate(order):
                qk(t)
                if k >= LAG: pv(order[k - LAG])
            for k in range(len(pieces)):
                piece(k)
                if k < LAG: pv(order[len(order) - LAG + k])
                for sidx, j in enumerate(vheads):
                    if k == dl[sidx]: vpv(j)
            outs = []
            for j in range(HPI):
                l = jnp.sum(jnp.concatenate(ls[j], axis=1), axis=0, keepdims=True)
                ok = jnp.minimum(ok, jnp.where((l >= L_LO) & (l <= L_HI), 1.0, 0.0))
                outs.append(accs[j] / l)
            oh_s[hh] = jnp.concatenate(outs, axis=0).T.astype(bf16)
            y_s[pl.ds(pl.multiple_of(hh * FR, FR), FR), :] = jnp.concatenate(y, axis=1)
            return ok

        @scope("attn")
        def attn():
            return lax.fori_loop(0, NI, heads, jnp.ones((1, TQ), f32))
        ok = attn()

        @pl.when(i == 0)
        def _():
            w_cp[5].wait()

        @scope("oblk")
        def finish():
            rows = pl.ds(pl.multiple_of(i * TQ, TQ), TQ)
            o = jnp.concatenate([oh_s[g] for g in range(NI)], axis=1)
            a = jnp.dot(o, wo_s[...], preferred_element_type=f32)
            o_ref[...] = (x_s[rows, :].astype(f32) + a + y_s[...]).astype(o_ref.dtype)
        finish()

        if fallback:
            @pl.when(jnp.min(ok) < 0.5)
            def _true_max_softmax():
                KB = 256
                def group(g, _):
                    outs = []
                    for j in range(HPI):
                        q = qT_s[i * H + g * HPI + j]
                        def chunk(c, carry):
                            m, l, acc = carry
                            ks = pl.ds(pl.multiple_of(c * KB, KB), KB)
                            s = jnp.dot(k_s[ks, 0:DH], q, preferred_element_type=f32)
                            m_new = jnp.maximum(m, jnp.max(s, axis=0, keepdims=True))
                            alpha = jnp.exp2(m - m_new)
                            p = jnp.exp2(s - m_new)
                            l = l * alpha + jnp.sum(p, axis=0, keepdims=True)
                            acc = acc * alpha + jnp.dot(vT_s[:, ks], p.astype(bf16), preferred_element_type=f32)
                            return m_new, l, acc
                        m, l, acc = lax.fori_loop(0, S // KB, chunk, (
                            jnp.full((1, TQ), -jnp.inf, f32), jnp.zeros((1, TQ), f32), jnp.zeros((DH, TQ), f32)))
                        outs.append(acc / l)
                    oh_s[g] = jnp.concatenate(outs, axis=0).T.astype(bf16)
                    return 0
                lax.fori_loop(0, NI, group, 0)
                finish()

    @jax.jit
    def run(A_x, A_wq, A_wk, A_wv, A_wo, B_x, B_w1, B_w2):
        x = A_x.reshape(S, D)
        out = pl.pallas_call(
            kernel,
            grid=(NT,),
            in_specs=[pl.BlockSpec(memory_space=pl.ANY)] * 7,
            out_specs=pl.BlockSpec((TQ, D), lambda i: (i, 0)),
            out_shape=jax.ShapeDtypeStruct((S, D), A_x.dtype),
            scratch_shapes=[
                pltpu.VMEM((S, D), bf16), pltpu.VMEM((D, D), bf16),
                pltpu.VMEM((D, D), bf16), pltpu.VMEM((D, F), bf16),
                pltpu.VMEM((F, D), bf16), pltpu.SemaphoreType.DMA((NT + 6,)),
                pltpu.VMEM((S, D), bf16),
                pltpu.VMEM((D + 2 * DH, D), bf16),
                pltpu.VMEM((S, 128), bf16),
                pltpu.VMEM((DH, S), bf16),
                pltpu.VMEM((DH, NC * KV, 128), f32),
                pltpu.VMEM((DH, KC, 128), f32),
                pltpu.VMEM((DH, TQ), f32),
                pltpu.VMEM((NT * H, DH, TQ), bf16),
                pltpu.VMEM((NT * H, DH, TQ), f32),
                pltpu.VMEM((NT * NI, HPI, TQ), f32),
                pltpu.VMEM((NI, TQ, GW), bf16),
                pltpu.VMEM((TQ, D), f32),
            ],
            compiler_params=pltpu.CompilerParams(
                dimension_semantics=("arbitrary",), vmem_limit_bytes=100 * 2 ** 20),
        )(x, A_wq, A_wk.T, A_wv.T, A_wo, B_w1, B_w2)
        return out.reshape(A_x.shape)
    return run


pallas_parallel_sum__grouped_kv_mqa__dense_activation_silu__prompt_kernel = make_kernel()
```

```python
import functools

import jax
import jax.numpy as jnp
from jax import lax
import jax.experimental.pallas as pl
import jax.experimental.pallas.tpu as pltpu

S, D, H, DH, F = 2048, 512, 32, 16, 1792
LOG2E = 1.4426950408889634
EPS = 1e-5
NT_DIMS = (((1,), (1,)), ((), ()))
L_LO, L_HI = 2.0 ** -40, 2.0 ** 40
MARGIN = 1.0 + 2.0 ** -6
TQ, KC, UW, KV = 512, 128, 128, 16
KM = KC - KV
NC, NU, NT, NF = S // KC, TQ // UW, S // TQ, F // 128
HW = TQ // 2
LAG = 2


def make_kernel(HPI=8, NVT=3, bounds=(0, 8, 16, 24), dl=(9, 17, 25), upos=(3, 6, 9, 12), vec=0):
    NI = H // HPI
    FR = TQ // NI
    GW = HPI * DH
    f32, bf16 = jnp.float32, jnp.bfloat16

    def kernel(x_hbm, wq_hbm, wkT_hbm, wvT_hbm, wo_hbm, w1_hbm, w2_hbm, o_ref,
               x_s, wq_s, wo_s, w1_s, w2_s, sems,
               xn_s, wT_s, k_s, vT_s, kb_s, kb2_s, zero_s, qT_s, qf_s, sh_s, oh_s, y_s):
        i = pl.program_id(0)
        x_cp = [pltpu.make_async_copy(x_hbm.at[pl.ds(t * TQ, TQ)], x_s.at[pl.ds(t * TQ, TQ)], sems.at[t])
                for t in range(NT)]
        w_cp = [pltpu.make_async_copy(src, dst, sems.at[NT + n]) for n, (src, dst) in enumerate(
            [(wq_hbm, wq_s), (wkT_hbm, wT_s.at[pl.ds(0, DH)]), (wvT_hbm, wT_s.at[pl.ds(DH, DH)]),
             (w1_hbm, w1_s), (w2_hbm, w2_s), (wo_hbm, wo_s)])]

        @pl.when(i == 0)
        def _prologue():
            x_cp[0].start()
            for cp in w_cp[:3]: cp.start()
            for cp in x_cp[1:]: cp.start()
            for cp in w_cp[3:]: cp.start()
            zero_s[...] = jnp.zeros(zero_s.shape, f32)
            hrow = lax.broadcasted_iota(jnp.int32, (H, D), 0)
            hcol = lax.broadcasted_iota(jnp.int32, (H, D), 1)
            blockdiag = jnp.where(hcol // DH == hrow, 1.0, 0.0).astype(bf16)
            kn2s, nqns = {}, {}

            def ln(t):
                rows = pl.ds(t * TQ, TQ)
                x = x_s[rows, :].astype(f32)
                xc = x - jnp.mean(x, axis=-1, keepdims=True)
                v = jnp.mean(xc * xc, axis=-1, keepdims=True)
                xn_s[rows, :] = (xc * lax.rsqrt(v + EPS)).astype(bf16)

            def proj(z):
                t, c0 = divmod(z * HW, TQ)
                res = lax.dot_general(wT_s[...], xn_s[z * HW:(z + 1) * HW, :], NT_DIMS,
                                      preferred_element_type=f32)
                vT_s[:, z * HW:(z + 1) * HW] = res[DH:2 * DH].astype(bf16)
                kT = res[0:DH].astype(bf16).astype(f32)
                kfull = jnp.concatenate([kT, jnp.zeros((128 - DH, HW), f32)], axis=0).T
                nk = HW // KC
                kv_rows = kfull.reshape(nk, KC, 128)[:, KM:, :].reshape(nk * KV, 128)
                for d in range(DH):
                    kb_s[d, z * nk * KV:(z + 1) * nk * KV, :] = jnp.broadcast_to(kv_rows[:, d:d + 1], (nk * KV, 128))
                if z == 2 * NT - 1:
                    for d in range(DH):
                        kb2_s[d] = jnp.broadcast_to(kfull[HW - KC:, d:d + 1], (KC, 128))
                kn2s[z] = jnp.sum(kT * kT, axis=0, keepdims=True)
                k_s[z * HW:(z + 1) * HW, :] = kfull.astype(bf16)
                qb = (res[2 * DH:] * (DH ** -0.5 * LOG2E)).astype(bf16)
                qT_s[t * H:(t + 1) * H, 0:DH, c0:c0 + HW] = qb.reshape(H, DH, HW)
                qf_s[t * H:(t + 1) * H, :, c0:c0 + HW] = qb.astype(f32).reshape(H, DH, HW)

            def norm(z):
                t, c0 = divmod(z * HW, TQ)
                qf = qf_s[t * H:(t + 1) * H, :, c0:c0 + HW].reshape(D, HW)
                qn2 = jnp.dot(blockdiag, (qf * qf).astype(bf16), preferred_element_type=f32)
                nqn = (jnp.sqrt(qn2) * -MARGIN).astype(bf16).astype(f32)
                row0 = lax.broadcasted_iota(jnp.int32, (DH, HW), 0) == 0
                for h in range(H):
                    qT_s[t * H + h, DH:, c0:c0 + HW] = jnp.where(
                        row0, jnp.broadcast_to(nqn[h:h + 1], (DH, HW)), 0.0).astype(bf16)
                nqns[z] = nqn

            x_cp[0].wait()
            ln(0)
            for cp in w_cp[:3]: cp.wait()
            wT_s[2 * DH:, :] = wq_s[...].astype(f32).T.astype(bf16)
            proj(0)
            x_cp[1].wait()
            proj(1); ln(1); norm(0); proj(2)
            x_cp[2].wait(); x_cp[3].wait()
            proj(3); ln(2); norm(1); ln(3); proj(4); norm(2); proj(5); norm(3); proj(6); norm(4); norm(5)
            proj(7); norm(6); norm(7)
            kn2 = functools.reduce(jnp.maximum, [kn2s[z] for z in range(2 * NT)])
            kmax = (jnp.sqrt(jnp.max(kn2, axis=1, keepdims=True)) * MARGIN).astype(bf16).astype(f32)
            k_s[:, DH:DH + 1] = jnp.broadcast_to(kmax, (S, 1)).astype(bf16)
            for z in range(2 * NT):
                t, c0 = divmod(z * HW, TQ)
                sh_s[t * NI:(t + 1) * NI, :, c0:c0 + HW] = (nqns[z] * kmax).reshape(NI, HPI, HW)
            for cp in w_cp[3:5]: cp.wait()

        def heads(hh, ok):
            hidx = [i * H + hh * HPI + j for j in range(HPI)]
            frows = pl.ds(pl.multiple_of(i * TQ + hh * FR, FR), FR)
            sidx = i * NI + hh
            n = HPI * NC
            accs = [zero_s[...] for _ in range(HPI)]
            ls = [[jnp.zeros((8, UW), f32) for _ in range(NU)] for _ in range(HPI)]
            always = zero_s[0:8, 0:UW] == 0.0
            ps, pvs, hact = {}, {}, {}
            y = [None] * 4

            @functools.cache
            def q_rows(j, u):
                cols = slice(u * UW, (u + 1) * UW)
                rows = [jnp.broadcast_to(qf_s[hidx[j], d:d + 1, cols], (KV, UW)) for d in range(DH)]
                return (jnp.stack(rows) if vec else rows), jnp.broadcast_to(sh_s[sidx, j:j + 1, cols], (KV, UW))

            @functools.cache
            def k_rows(last, g):
                ref = kb2_s if last else kb_s
                if vec: return ref[:, g * KV:(g + 1) * KV, :]
                return [ref[d, g * KV:(g + 1) * KV, :] for d in range(DH)]

            def unit(j, last, g, u, anchor=None):
                if anchor is not None:
                    ls[j][u] = jnp.where(always, ls[j][u], anchor)
                q, sv = q_rows(j, u)
                k = k_rows(last, g)
                if vec == 1:
                    prod = k * q
                    for d in range(DH): sv = sv + prod[d]
                elif vec == 2:
                    sv = sv + jnp.sum(k * q, axis=0)
                else:
                    for d in range(DH): sv = sv + k[d] * q[d]
                p = jnp.exp2(sv)
                ls[j][u] = ls[j][u] + p[0:8] + p[8:16]
                pvs[(j, last, g, u)] = p

            def vrows(j, last, g):
                return jnp.concatenate([pvs.pop((j, last, g, u)) for u in range(NU)], axis=1)

            def qk(t):
                j, c = divmod(t, NC)
                p = jnp.exp2(jnp.dot(k_s[c * KC:c * KC + KM, 0:2 * DH], qT_s[hidx[j]], preferred_element_type=f32))
                for r in range(KM // 8):
                    for u in range(NU):
                        ls[j][u] = ls[j][u] + p[r * 8:(r + 1) * 8, u * UW:(u + 1) * UW]
                    if r in upos:
                        unit(j, False, c, upos.index(r))
                ps[t] = p

            def pv(j, c, parts):
                p = jnp.concatenate(parts, axis=0).astype(bf16)
                accs[j] = accs[j] + jnp.dot(vT_s[:, c * KC:(c + 1) * KC], p, preferred_element_type=f32)

            def pv_reg(t):
                j, c = divmod(t, NC)
                pv(j, c, [ps.pop(t), vrows(j, False, c)])

            w2p = [[('w2', (4 * g, 4 * g + 4, nn, nn + 1)) for nn in range(4)] for g in range(3)]
            w2p.append([('w2', (12, 14, 0, 2)), ('w2', (12, 14, 2, 4))])
            w1p = [('w1', m) for m in range(NF)]
            pieces = w1p[0:5]
            for k in range(4): pieces += [w2p[0][k], w1p[5 + k]]
            for k in range(4): pieces += [w2p[1][k], w1p[9 + k]]
            pieces += [w2p[2][0], w1p[13]] + w2p[2][1:] + w2p[3]
            vheads = list(range(HPI - NVT, HPI))
            where2 = {}
            for s_, j in enumerate(vheads):
                slots = [divmod(q, FR // 8) for q in range(int(bounds[s_] * FR // 8), int(bounds[s_ + 1] * FR // 8))]
                us = [(j, True, g, u) for g in range(KC // KV) for u in range(NU)]
                for k, un in enumerate(us):
                    where2[slots[((2 * k + 1) * len(slots)) // (2 * len(us))]] = un

            def piece(k):
                kind, a = pieces[k]
                if kind == 'w1':
                    res = jnp.dot(xn_s[frows, :], w1_s[:, a * 128:(a + 1) * 128], preferred_element_type=f32)
                else:
                    k0, k1, n0, n1 = a
                    res = jnp.dot(jnp.concatenate([hact[kk] for kk in range(k0, k1)], axis=1),
                                  w2_s[k0 * 128:k1 * 128, n0 * 128:n1 * 128], preferred_element_type=f32)
                for r in range(FR // 8):
                    if (k, r) in where2:
                        unit(*where2[(k, r)], anchor=res[r * 8:(r + 1) * 8, 0:UW])
                if kind == 'w1':
                    hm = 0.5 * res
                    hact[a] = (hm + hm * jnp.tanh(hm)).astype(bf16)
                else:
                    for nn in range(n0, n1):
                        pn = res[:, (nn - n0) * 128:(nn - n0 + 1) * 128]
                        y[nn] = pn if y[nn] is None else y[nn] + pn

            order = [t for t in range(n) if not (t % NC == NC - 1 and t // NC in vheads)]
            for k, t in enumerate(order):
                qk(t)
                if k >= LAG: pv_reg(order[k - LAG])
            for k in range(len(pieces)):
                piece(k)
                if k < LAG: pv_reg(order[len(order) - LAG + k])
                if k in dl:
                    j = vheads[dl.index(k)]
                    pv(j, NC - 1, [vrows(j, True, g) for g in range(KC // KV)])
            outs = []
            for j in range(HPI):
                l = jnp.sum(jnp.concatenate(ls[j], axis=1), axis=0, keepdims=True)
                ok = jnp.minimum(ok, jnp.where((l >= L_LO) & (l <= L_HI), 1.0, 0.0))
                outs.append(accs[j] / l)
            oh_s[hh] = jnp.concatenate(outs, axis=0).T.astype(bf16)
            y_s[pl.ds(pl.multiple_of(hh * FR, FR), FR), :] = jnp.concatenate(y, axis=1)
            return ok

        ok = lax.fori_loop(0, NI, heads, jnp.ones((1, TQ), f32))

        @pl.when(i == 0)
        def _():
            w_cp[5].wait()

        def finish():
            rows = pl.ds(pl.multiple_of(i * TQ, TQ), TQ)
            o = jnp.concatenate([oh_s[g] for g in range(NI)], axis=1)
            a = jnp.dot(o, wo_s[...], preferred_element_type=f32)
            o_ref[...] = (x_s[rows, :].astype(f32) + a + y_s[...]).astype(o_ref.dtype)
        finish()

        @pl.when(jnp.min(ok) < 0.5)
        def _true_max_softmax():
            KB = 256

            def group(g, _):
                outs = []
                for j in range(HPI):
                    q = qT_s[i * H + g * HPI + j, 0:DH, :]

                    def chunk(c, carry):
                        m, l, acc = carry
                        ks = pl.ds(pl.multiple_of(c * KB, KB), KB)
                        s = jnp.dot(k_s[ks, 0:DH], q, preferred_element_type=f32)
                        m_new = jnp.maximum(m, jnp.max(s, axis=0, keepdims=True))
                        alpha = jnp.exp2(m - m_new)
                        p = jnp.exp2(s - m_new)
                        l = l * alpha + jnp.sum(p, axis=0, keepdims=True)
                        acc = acc * alpha + jnp.dot(vT_s[:, ks], p.astype(bf16), preferred_element_type=f32)
                        return m_new, l, acc
                    m, l, acc = lax.fori_loop(0, S // KB, chunk, (
                        jnp.full((1, TQ), -jnp.inf, f32), jnp.zeros((1, TQ), f32), jnp.zeros((DH, TQ), f32)))
                    outs.append(acc / l)
                oh_s[g] = jnp.concatenate(outs, axis=0).T.astype(bf16)
                return 0
            lax.fori_loop(0, NI, group, 0)
            finish()

    @jax.jit
    def run(A_x, A_wq, A_wk, A_wv, A_wo, B_x, B_w1, B_w2):
        out = pl.pallas_call(
            kernel,
            grid=(NT,),
            in_specs=[pl.BlockSpec(memory_space=pl.ANY)] * 7,
            out_specs=pl.BlockSpec((TQ, D), lambda i: (i, 0)),
            out_shape=jax.ShapeDtypeStruct((S, D), A_x.dtype),
            scratch_shapes=[
                pltpu.VMEM((S, D), bf16), pltpu.VMEM((D, D), bf16),
                pltpu.VMEM((D, D), bf16), pltpu.VMEM((D, F), bf16),
                pltpu.VMEM((F, D), bf16), pltpu.SemaphoreType.DMA((NT + 6,)),
                pltpu.VMEM((S, D), bf16),
                pltpu.VMEM((D + 2 * DH, D), bf16),
                pltpu.VMEM((S, 128), bf16),
                pltpu.VMEM((DH, S), bf16),
                pltpu.VMEM((DH, NC * KV, 128), f32),
                pltpu.VMEM((DH, KC, 128), f32),
                pltpu.VMEM((DH, TQ), f32),
                pltpu.VMEM((NT * H, 2 * DH, TQ), bf16),
                pltpu.VMEM((NT * H, DH, TQ), f32),
                pltpu.VMEM((NT * NI, HPI, TQ), f32),
                pltpu.VMEM((NI, TQ, GW), bf16),
                pltpu.VMEM((TQ, D), f32),
            ],
            compiler_params=pltpu.CompilerParams(
                dimension_semantics=("arbitrary",), vmem_limit_bytes=100 * 2 ** 20),
        )(A_x.reshape(S, D), A_wq, A_wk.T, A_wv.T, A_wo, B_w1, B_w2)
        return out.reshape(A_x.shape)
    return run


pallas_parallel_sum__grouped_kv_mqa__dense_activation_silu__prompt_kernel = make_kernel()
```

```python
import functools

import jax
import jax.numpy as jnp
from jax import lax
import jax.experimental.pallas as pl
import jax.experimental.pallas.tpu as pltpu

S, D, H, DH, F = 2048, 512, 32, 16, 1792
LOG2E = 1.4426950408889634
EPS = 1e-5
NT_DIMS = (((1,), (1,)), ((), ()))
L_LO, L_HI = 2.0 ** -40, 2.0 ** 12
MARGIN = 1.0 + 2.0 ** -6
TQ, KC, UW, KV = 512, 128, 128, 16
KM = KC - KV
NC, NU, NT, NF = S // KC, TQ // UW, S // TQ, F // 128
HW = TQ // 2
LAG = 2


def make_kernel(HPI=8, NVT=3, bounds=(0, 8, 16, 24), dl=(9, 17, 25), upos=(3, 6, 9, 12), vec=0, NO=4):
    NI = H // HPI
    FR = TQ // NI
    GW = HPI * DH
    f32, bf16 = jnp.float32, jnp.bfloat16

    def kernel(x_hbm, wq_hbm, wkT_hbm, wvT_hbm, wo_hbm, w1_hbm, w2_hbm, o_hbm,
               x_s, wq_s, wo_s, w1_s, w2_s, sems,
               xn_s, wT_s, k_s, vT_s, kb_s, kb2_s, zero_s, qT_s, qf_s, sh_s, oh_s, y_s, out_s, osems):
        i = pl.program_id(0)
        x_cp = [pltpu.make_async_copy(x_hbm.at[pl.ds(t * TQ, TQ)], x_s.at[pl.ds(t * TQ, TQ)], sems.at[t])
                for t in range(NT)]
        w_cp = [pltpu.make_async_copy(src, dst, sems.at[NT + n]) for n, (src, dst) in enumerate(
            [(wq_hbm, wq_s), (wkT_hbm, wT_s.at[pl.ds(0, DH)]), (wvT_hbm, wT_s.at[pl.ds(DH, DH)]),
             (w1_hbm, w1_s), (w2_hbm, w2_s), (wo_hbm, wo_s)])]

        @pl.when(i == 0)
        def _prologue():
            x_cp[0].start()
            for cp in w_cp[:3]: cp.start()
            for cp in x_cp[1:]: cp.start()
            for cp in w_cp[3:]: cp.start()
            zero_s[...] = jnp.zeros(zero_s.shape, f32)
            hrow = lax.broadcasted_iota(jnp.int32, (H, D), 0)
            hcol = lax.broadcasted_iota(jnp.int32, (H, D), 1)
            blockdiag = jnp.where(hcol // DH == hrow, 1.0, 0.0).astype(bf16)
            kn2s, nqns = {}, {}

            def ln(t):
                rows = pl.ds(t * TQ, TQ)
                x = x_s[rows, :].astype(f32)
                xc = x - jnp.mean(x, axis=-1, keepdims=True)
                v = jnp.mean(xc * xc, axis=-1, keepdims=True)
                xn_s[rows, :] = (xc * lax.rsqrt(v + EPS)).astype(bf16)

            def proj(z):
                t, c0 = divmod(z * HW, TQ)
                res = lax.dot_general(wT_s[...], xn_s[z * HW:(z + 1) * HW, :], NT_DIMS,
                                      preferred_element_type=f32)
                vT_s[:, z * HW:(z + 1) * HW] = res[DH:2 * DH].astype(bf16)
                kT = res[0:DH].astype(bf16).astype(f32)
                kfull = jnp.concatenate([kT, jnp.zeros((128 - DH, HW), f32)], axis=0).T
                nk = HW // KC
                kv_rows = kfull.reshape(nk, KC, 128)[:, KM:, :].reshape(nk * KV, 128)
                for d in range(DH):
                    kb_s[d, z * nk * KV:(z + 1) * nk * KV, :] = jnp.broadcast_to(kv_rows[:, d:d + 1], (nk * KV, 128))
                if z == 2 * NT - 1:
                    for d in range(DH):
                        kb2_s[d] = jnp.broadcast_to(kfull[HW - KC:, d:d + 1], (KC, 128))
                kn2s[z] = jnp.sum(kT * kT, axis=0, keepdims=True)
                k_s[z * HW:(z + 1) * HW, :] = kfull.astype(bf16)
                qb = (res[2 * DH:] * (DH ** -0.5 * LOG2E)).astype(bf16)
                qT_s[t * H:(t + 1) * H, 0:DH, c0:c0 + HW] = qb.reshape(H, DH, HW)
                qf_s[t * H:(t + 1) * H, :, c0:c0 + HW] = qb.astype(f32).reshape(H, DH, HW)

            def norm(z):
                t, c0 = divmod(z * HW, TQ)
                qf = qf_s[t * H:(t + 1) * H, :, c0:c0 + HW].reshape(D, HW)
                qn2 = jnp.dot(blockdiag, (qf * qf).astype(bf16), preferred_element_type=f32)
                nqn = (jnp.sqrt(qn2) * -MARGIN).astype(bf16).astype(f32)
                row0 = lax.broadcasted_iota(jnp.int32, (DH, HW), 0) == 0
                for h in range(H):
                    qT_s[t * H + h, DH:, c0:c0 + HW] = jnp.where(
                        row0, jnp.broadcast_to(nqn[h:h + 1], (DH, HW)), 0.0).astype(bf16)
                nqns[z] = nqn

            x_cp[0].wait()
            ln(0)
            for cp in w_cp[:3]: cp.wait()
            wT_s[2 * DH:, :] = wq_s[...].astype(f32).T.astype(bf16)
            proj(0)
            x_cp[1].wait()
            proj(1); ln(1); norm(0); proj(2)
            x_cp[2].wait(); x_cp[3].wait()
            proj(3); ln(2); norm(1); ln(3); proj(4); norm(2); proj(5); norm(3); proj(6); norm(4); norm(5)
            proj(7); norm(6); norm(7)
            kn2 = functools.reduce(jnp.maximum, [kn2s[z] for z in range(2 * NT)])
            kmax = (jnp.sqrt(jnp.max(kn2, axis=1, keepdims=True)) * MARGIN).astype(bf16).astype(f32)
            k_s[:, DH:DH + 1] = jnp.broadcast_to(kmax, (S, 1)).astype(bf16)
            for z in range(2 * NT):
                t, c0 = divmod(z * HW, TQ)
                sh_s[t * NI:(t + 1) * NI, :, c0:c0 + HW] = (nqns[z] * kmax).reshape(NI, HPI, HW)
            for cp in w_cp[3:5]: cp.wait()

        def heads(hh, ok):
            hidx = [i * H + hh * HPI + j for j in range(HPI)]
            frows = pl.ds(pl.multiple_of(i * TQ + hh * FR, FR), FR)
            sidx = i * NI + hh
            n = HPI * NC
            accs = [zero_s[...] for _ in range(HPI)]
            ls = [[jnp.zeros((8, UW), f32) for _ in range(NU)] for _ in range(HPI)]
            always = zero_s[0:8, 0:UW] == 0.0
            ps, pvs, hact = {}, {}, {}
            y = [None] * 4

            @functools.cache
            def q_rows(j, u):
                cols = slice(u * UW, (u + 1) * UW)
                rows = [jnp.broadcast_to(qf_s[hidx[j], d:d + 1, cols], (KV, UW)) for d in range(DH)]
                return (jnp.stack(rows) if vec else rows), jnp.broadcast_to(sh_s[sidx, j:j + 1, cols], (KV, UW))

            @functools.cache
            def k_rows(last, g):
                ref = kb2_s if last else kb_s
                if vec: return ref[:, g * KV:(g + 1) * KV, :]
                return [ref[d, g * KV:(g + 1) * KV, :] for d in range(DH)]

            def unit(j, last, g, u, anchor=None):
                if anchor is not None:
                    ls[j][u] = jnp.where(always, ls[j][u], anchor)
                q, sv = q_rows(j, u)
                k = k_rows(last, g)
                if vec == 1:
                    prod = k * q
                    for d in range(DH): sv = sv + prod[d]
                elif vec == 2:
                    sv = sv + jnp.sum(k * q, axis=0)
                else:
                    for d in range(DH): sv = sv + k[d] * q[d]
                p = jnp.exp2(sv)
                ls[j][u] = ls[j][u] + p[0:8] + p[8:16]
                pvs[(j, last, g, u)] = p

            def vrows(j, last, g):
                return jnp.concatenate([pvs.pop((j, last, g, u)) for u in range(NU)], axis=1)

            def qk(t):
                j, c = divmod(t, NC)
                p = jnp.exp2(jnp.dot(k_s[c * KC:c * KC + KM, 0:2 * DH], qT_s[hidx[j]], preferred_element_type=f32))
                for r in range(KM // 8):
                    for u in range(NU):
                        ls[j][u] = ls[j][u] + p[r * 8:(r + 1) * 8, u * UW:(u + 1) * UW]
                    if r in upos:
                        unit(j, False, c, upos.index(r))
                ps[t] = p

            def pv(j, c, parts):
                p = jnp.concatenate(parts, axis=0).astype(bf16)
                accs[j] = accs[j] + jnp.dot(vT_s[:, c * KC:(c + 1) * KC], p, preferred_element_type=f32)

            def pv_reg(t):
                j, c = divmod(t, NC)
                pv(j, c, [ps.pop(t), vrows(j, False, c)])

            w2p = [[('w2', (4 * g, 4 * g + 4, nn, nn + 1)) for nn in range(4)] for g in range(3)]
            w2p.append([('w2', (12, 14, 0, 2)), ('w2', (12, 14, 2, 4))])
            w1p = [('w1', m) for m in range(NF)]
            pieces = w1p[0:5]
            for k in range(4): pieces += [w2p[0][k], w1p[5 + k]]
            for k in range(4): pieces += [w2p[1][k], w1p[9 + k]]
            pieces += [w2p[2][0], w1p[13]] + w2p[2][1:] + w2p[3]
            vheads = list(range(HPI - NVT, HPI))
            where2 = {}
            for s_, j in enumerate(vheads):
                slots = [divmod(q, FR // 8) for q in range(int(bounds[s_] * FR // 8), int(bounds[s_ + 1] * FR // 8))]
                us = [(j, True, g, u) for g in range(KC // KV) for u in range(NU)]
                for k, un in enumerate(us):
                    where2[slots[((2 * k + 1) * len(slots)) // (2 * len(us))]] = un

            def piece(k):
                kind, a = pieces[k]
                if kind == 'w1':
                    res = jnp.dot(xn_s[frows, :], w1_s[:, a * 128:(a + 1) * 128], preferred_element_type=f32)
                else:
                    k0, k1, n0, n1 = a
                    res = jnp.dot(jnp.concatenate([hact[kk] for kk in range(k0, k1)], axis=1),
                                  w2_s[k0 * 128:k1 * 128, n0 * 128:n1 * 128], preferred_element_type=f32)
                for r in range(FR // 8):
                    if (k, r) in where2:
                        unit(*where2[(k, r)], anchor=res[r * 8:(r + 1) * 8, 0:UW])
                if kind == 'w1':
                    hm = 0.5 * res
                    hact[a] = (hm + hm * jnp.tanh(hm)).astype(bf16)
                else:
                    for nn in range(n0, n1):
                        pn = res[:, (nn - n0) * 128:(nn - n0 + 1) * 128]
                        y[nn] = pn if y[nn] is None else y[nn] + pn

            order = [t for t in range(n) if not (t % NC == NC - 1 and t // NC in vheads)]
            for k, t in enumerate(order):
                qk(t)
                if k >= LAG: pv_reg(order[k - LAG])
            for k in range(len(pieces)):
                piece(k)
                if k < LAG: pv_reg(order[len(order) - LAG + k])
                if k in dl:
                    j = vheads[dl.index(k)]
                    pv(j, NC - 1, [vrows(j, True, g) for g in range(KC // KV)])
            outs = []
            for j in range(HPI):
                l = jnp.sum(jnp.concatenate(ls[j], axis=1), axis=0, keepdims=True)
                ok = jnp.minimum(ok, jnp.where((l >= L_LO) & (l <= L_HI), 1.0, 0.0))
                outs.append(accs[j] / l)
            oh_s[hh] = jnp.concatenate(outs, axis=0).T.astype(bf16)
            y_s[pl.ds(pl.multiple_of(hh * FR, FR), FR), :] = jnp.concatenate(y, axis=1)
            return ok

        ok = lax.fori_loop(0, NI, heads, jnp.ones((1, TQ), f32))

        OR = TQ // NO

        def o_cp(t, r):
            return pltpu.make_async_copy(out_s.at[pl.ds(r * OR, OR)],
                                         o_hbm.at[pl.ds(pl.multiple_of(t * TQ + r * OR, OR), OR)], osems.at[r])

        @pl.when(i == 0)
        def _():
            w_cp[5].wait()

        @pl.when(i > 0)
        def _():
            for r in range(NO): o_cp(i - 1, r).wait()

        def finish():
            for r in range(NO):
                rows = pl.ds(pl.multiple_of(i * TQ + r * OR, OR), OR)
                o = jnp.concatenate([oh_s[g, r * OR:(r + 1) * OR, :] for g in range(NI)], axis=1)
                a = jnp.dot(o, wo_s[...], preferred_element_type=f32)
                out_s[r * OR:(r + 1) * OR, :] = (
                    x_s[rows, :].astype(f32) + a + y_s[r * OR:(r + 1) * OR, :]).astype(out_s.dtype)
                o_cp(i, r).start()
        finish()

        @pl.when(jnp.min(ok) < 0.5)
        def _true_max_softmax():
            KB = 256

            def group(g, _):
                outs = []
                for j in range(HPI):
                    q = qT_s[i * H + g * HPI + j, 0:DH, :]

                    def chunk(c, carry):
                        m, l, acc = carry
                        ks = pl.ds(pl.multiple_of(c * KB, KB), KB)
                        s = jnp.dot(k_s[ks, 0:DH], q, preferred_element_type=f32)
                        m_new = jnp.maximum(m, jnp.max(s, axis=0, keepdims=True))
                        alpha = jnp.exp2(m - m_new)
                        p = jnp.exp2(s - m_new)
                        l = l * alpha + jnp.sum(p, axis=0, keepdims=True)
                        acc = acc * alpha + jnp.dot(vT_s[:, ks], p.astype(bf16), preferred_element_type=f32)
                        return m_new, l, acc
                    m, l, acc = lax.fori_loop(0, S // KB, chunk, (
                        jnp.full((1, TQ), -jnp.inf, f32), jnp.zeros((1, TQ), f32), jnp.zeros((DH, TQ), f32)))
                    outs.append(acc / l)
                oh_s[g] = jnp.concatenate(outs, axis=0).T.astype(bf16)
                return 0
            lax.fori_loop(0, NI, group, 0)
            for r in range(NO): o_cp(i, r).wait()
            finish()

        @pl.when(i == NT - 1)
        def _():
            for r in range(NO): o_cp(i, r).wait()

    @jax.jit
    def run(A_x, A_wq, A_wk, A_wv, A_wo, B_x, B_w1, B_w2):
        out = pl.pallas_call(
            kernel,
            grid=(NT,),
            in_specs=[pl.BlockSpec(memory_space=pl.ANY)] * 7,
            out_specs=pl.BlockSpec(memory_space=pl.ANY),
            out_shape=jax.ShapeDtypeStruct((S, D), A_x.dtype),
            scratch_shapes=[
                pltpu.VMEM((S, D), bf16), pltpu.VMEM((D, D), bf16),
                pltpu.VMEM((D, D), bf16), pltpu.VMEM((D, F), bf16),
                pltpu.VMEM((F, D), bf16), pltpu.SemaphoreType.DMA((NT + 6,)),
                pltpu.VMEM((S, D), bf16),
                pltpu.VMEM((D + 2 * DH, D), bf16),
                pltpu.VMEM((S, 128), bf16),
                pltpu.VMEM((DH, S), bf16),
                pltpu.VMEM((DH, NC * KV, 128), f32),
                pltpu.VMEM((DH, KC, 128), f32),
                pltpu.VMEM((DH, TQ), f32),
                pltpu.VMEM((NT * H, 2 * DH, TQ), bf16),
                pltpu.VMEM((NT * H, DH, TQ), f32),
                pltpu.VMEM((NT * NI, HPI, TQ), f32),
                pltpu.VMEM((NI, TQ, GW), bf16),
                pltpu.VMEM((TQ, D), f32),
                pltpu.VMEM((TQ, D), bf16),
                pltpu.SemaphoreType.DMA((NO,)),
            ],
            compiler_params=pltpu.CompilerParams(
                dimension_semantics=("arbitrary",), vmem_limit_bytes=100 * 2 ** 20),
        )(A_x.reshape(S, D), A_wq, A_wk.T, A_wv.T, A_wo, B_w1, B_w2)
        return out.reshape(A_x.shape)
    return run


pallas_parallel_sum__grouped_kv_mqa__dense_activation_silu__prompt_kernel = make_kernel()
```

```python
import functools

import jax
import jax.numpy as jnp
from jax import lax
import jax.experimental.pallas as pl
import jax.experimental.pallas.tpu as pltpu

S, D, H, DH, F = 2048, 512, 32, 16, 1792
LOG2E = 1.4426950408889634
EPS = 1e-5
NT_DIMS = (((1,), (1,)), ((), ()))
L_LO, L_HI = 2.0 ** -40, 2.0 ** 12
MARGIN = 1.0 + 2.0 ** -6

TQ, KC, UW, KV = 512, 128, 128, 16
KM = KC - KV
NC, NU, NT, NF = S // KC, TQ // UW, S // TQ, F // 128
HW = TQ // 2
LAG = 2
HPI = 8
NI = H // HPI
FR = TQ // NI
GW = HPI * DH
NO = 4
OR = TQ // NO
UPOS = (3, 6, 9, 12)
VHEADS = (5, 6, 7)
VBOUNDS = (0, 8, 16, 24)
VDUE = (9, 17, 25)

f32, bf16 = jnp.float32, jnp.bfloat16


def _ffn_pieces():
    w2p = [[('w2', (4 * g, 4 * g + 4, n, n + 1)) for n in range(4)] for g in range(3)]
    w2p.append([('w2', (12, 14, 0, 2)), ('w2', (12, 14, 2, 4))])
    w1p = [('w1', m) for m in range(NF)]
    pieces = w1p[0:5]
    for k in range(4):
        pieces += [w2p[0][k], w1p[5 + k]]
    for k in range(4):
        pieces += [w2p[1][k], w1p[9 + k]]
    return pieces + [w2p[2][0], w1p[13]] + w2p[2][1:] + w2p[3]


def _vunit_slots():
    out = {}
    for s, j in enumerate(VHEADS):
        slots = [divmod(q, FR // 8) for q in range(VBOUNDS[s] * FR // 8, VBOUNDS[s + 1] * FR // 8)]
        units = [(j, True, g, u) for g in range(KC // KV) for u in range(NU)]
        for k, un in enumerate(units):
            out[slots[((2 * k + 1) * len(slots)) // (2 * len(units))]] = un
    return out


def _kernel(x_hbm, wq_hbm, wkT_hbm, wvT_hbm, wo_hbm, w1_hbm, w2_hbm, o_hbm,
            x_s, wq_s, wo_s, w1_s, w2_s, sems,
            xn_s, wT_s, k_s, vT_s, kb_s, kb2_s, zero_s, qT_s, qf_s, sh_s, oh_s, y_s, out_s, osems):
    i = pl.program_id(0)
    x_cp = [pltpu.make_async_copy(x_hbm.at[pl.ds(t * TQ, TQ)], x_s.at[pl.ds(t * TQ, TQ)], sems.at[t])
            for t in range(NT)]
    w_cp = [pltpu.make_async_copy(src, dst, sems.at[NT + n]) for n, (src, dst) in enumerate(
        [(wq_hbm, wq_s), (wkT_hbm, wT_s.at[pl.ds(0, DH)]), (wvT_hbm, wT_s.at[pl.ds(DH, DH)]),
         (w1_hbm, w1_s), (w2_hbm, w2_s), (wo_hbm, wo_s)])]

    def o_cp(t, r):
        return pltpu.make_async_copy(out_s.at[pl.ds(r * OR, OR)],
                                     o_hbm.at[pl.ds(pl.multiple_of(t * TQ + r * OR, OR), OR)], osems.at[r])

    @pl.when(i == 0)
    def _prologue():
        x_cp[0].start()
        for cp in w_cp[:3] + x_cp[1:] + w_cp[3:]:
            cp.start()
        zero_s[...] = jnp.zeros(zero_s.shape, f32)
        hrow = lax.broadcasted_iota(jnp.int32, (H, D), 0)
        hcol = lax.broadcasted_iota(jnp.int32, (H, D), 1)
        blockdiag = jnp.where(hcol // DH == hrow, 1.0, 0.0).astype(bf16)
        kn2s, nqns = {}, {}

        def ln(t):
            rows = pl.ds(t * TQ, TQ)
            x = x_s[rows, :].astype(f32)
            xc = x - jnp.mean(x, axis=-1, keepdims=True)
            v = jnp.mean(xc * xc, axis=-1, keepdims=True)
            xn_s[rows, :] = (xc * lax.rsqrt(v + EPS)).astype(bf16)

        def proj(z):
            t, c0 = divmod(z * HW, TQ)
            res = lax.dot_general(wT_s[...], xn_s[z * HW:(z + 1) * HW, :], NT_DIMS,
                                  preferred_element_type=f32)
            vT_s[:, z * HW:(z + 1) * HW] = res[DH:2 * DH].astype(bf16)
            kT = res[0:DH].astype(bf16).astype(f32)
            kfull = jnp.concatenate([kT, jnp.zeros((128 - DH, HW), f32)], axis=0).T
            nk = HW // KC
            kv_rows = kfull.reshape(nk, KC, 128)[:, KM:, :].reshape(nk * KV, 128)
            for d in range(DH):
                kb_s[d, z * nk * KV:(z + 1) * nk * KV, :] = jnp.broadcast_to(kv_rows[:, d:d + 1], (nk * KV, 128))
            if z == 2 * NT - 1:
                for d in range(DH):
                    kb2_s[d] = jnp.broadcast_to(kfull[HW - KC:, d:d + 1], (KC, 128))
            kn2s[z] = jnp.sum(kT * kT, axis=0, keepdims=True)
            k_s[z * HW:(z + 1) * HW, :] = kfull.astype(bf16)
            qb = (res[2 * DH:] * (DH ** -0.5 * LOG2E)).astype(bf16)
            qT_s[t * H:(t + 1) * H, 0:DH, c0:c0 + HW] = qb.reshape(H, DH, HW)
            qf_s[t * H:(t + 1) * H, :, c0:c0 + HW] = qb.astype(f32).reshape(H, DH, HW)

        def norm(z):
            t, c0 = divmod(z * HW, TQ)
            qf = qf_s[t * H:(t + 1) * H, :, c0:c0 + HW].reshape(D, HW)
            qn2 = jnp.dot(blockdiag, (qf * qf).astype(bf16), preferred_element_type=f32)
            nqn = (jnp.sqrt(qn2) * -MARGIN).astype(bf16).astype(f32)
            row0 = lax.broadcasted_iota(jnp.int32, (DH, HW), 0) == 0
            for h in range(H):
                qT_s[t * H + h, DH:, c0:c0 + HW] = jnp.where(
                    row0, jnp.broadcast_to(nqn[h:h + 1], (DH, HW)), 0.0).astype(bf16)
            nqns[z] = nqn

        x_cp[0].wait()
        ln(0)
        for cp in w_cp[:3]:
            cp.wait()
        wT_s[2 * DH:, :] = wq_s[...].astype(f32).T.astype(bf16)
        proj(0)
        x_cp[1].wait()
        proj(1); ln(1); norm(0); proj(2)
        x_cp[2].wait()
        x_cp[3].wait()
        proj(3); ln(2); norm(1); ln(3); proj(4); norm(2); proj(5); norm(3); proj(6); norm(4); norm(5)
        proj(7); norm(6); norm(7)
        kn2 = functools.reduce(jnp.maximum, [kn2s[z] for z in range(2 * NT)])
        kmax = (jnp.sqrt(jnp.max(kn2, axis=1, keepdims=True)) * MARGIN).astype(bf16).astype(f32)
        k_s[:, DH:DH + 1] = jnp.broadcast_to(kmax, (S, 1)).astype(bf16)
        for z in range(2 * NT):
            t, c0 = divmod(z * HW, TQ)
            sh_s[t * NI:(t + 1) * NI, :, c0:c0 + HW] = (nqns[z] * kmax).reshape(NI, HPI, HW)
        for cp in w_cp[3:5]:
            cp.wait()

    pieces, vslots = _ffn_pieces(), _vunit_slots()

    def heads(hh, ok):
        hidx = [i * H + hh * HPI + j for j in range(HPI)]
        frows = pl.ds(pl.multiple_of(i * TQ + hh * FR, FR), FR)
        sidx = i * NI + hh
        accs = [zero_s[...] for _ in range(HPI)]
        ls = [[jnp.zeros((8, UW), f32) for _ in range(NU)] for _ in range(HPI)]
        always = zero_s[0:8, 0:UW] == 0.0
        ps, pvs, hact = {}, {}, {}
        y = [None] * (D // 128)

        @functools.cache
        def q_rows(j, u):
            cols = slice(u * UW, (u + 1) * UW)
            return ([jnp.broadcast_to(qf_s[hidx[j], d:d + 1, cols], (KV, UW)) for d in range(DH)],
                    jnp.broadcast_to(sh_s[sidx, j:j + 1, cols], (KV, UW)))

        @functools.cache
        def k_rows(last, g):
            ref = kb2_s if last else kb_s
            return [ref[d, g * KV:(g + 1) * KV, :] for d in range(DH)]

        def unit(j, last, g, u, anchor=None):
            if anchor is not None:
                ls[j][u] = jnp.where(always, ls[j][u], anchor)
            q, sv = q_rows(j, u)
            k = k_rows(last, g)
            for d in range(DH):
                sv = sv + k[d] * q[d]
            p = jnp.exp2(sv)
            ls[j][u] = ls[j][u] + p[0:8] + p[8:16]
            pvs[(j, last, g, u)] = p

        def vrows(j, last, g):
            return jnp.concatenate([pvs.pop((j, last, g, u)) for u in range(NU)], axis=1)

        def qk(t):
            j, c = divmod(t, NC)
            p = jnp.exp2(jnp.dot(k_s[c * KC:c * KC + KM, 0:2 * DH], qT_s[hidx[j]], preferred_element_type=f32))
            for r in range(KM // 8):
                for u in range(NU):
                    ls[j][u] = ls[j][u] + p[r * 8:(r + 1) * 8, u * UW:(u + 1) * UW]
                if r in UPOS:
                    unit(j, False, c, UPOS.index(r))
            ps[t] = p

        def pv(j, c, parts):
            p = jnp.concatenate(parts, axis=0).astype(bf16)
            accs[j] = accs[j] + jnp.dot(vT_s[:, c * KC:(c + 1) * KC], p, preferred_element_type=f32)

        def pv_reg(t):
            j, c = divmod(t, NC)
            pv(j, c, [ps.pop(t), vrows(j, False, c)])

        def piece(k):
            kind, a = pieces[k]
            if kind == 'w1':
                res = jnp.dot(xn_s[frows, :], w1_s[:, a * 128:(a + 1) * 128], preferred_element_type=f32)
            else:
                k0, k1, n0, n1 = a
                res = jnp.dot(jnp.concatenate([hact[kk] for kk in range(k0, k1)], axis=1),
                              w2_s[k0 * 128:k1 * 128, n0 * 128:n1 * 128], preferred_element_type=f32)
            for r in range(FR // 8):
                if (k, r) in vslots:
                    unit(*vslots[(k, r)], anchor=res[r * 8:(r + 1) * 8, 0:UW])
            if kind == 'w1':
                hm = 0.5 * res
                hact[a] = (hm + hm * jnp.tanh(hm)).astype(bf16)
            else:
                for n in range(n0, n1):
                    pn = res[:, (n - n0) * 128:(n - n0 + 1) * 128]
                    y[n] = pn if y[n] is None else y[n] + pn

        order = [t for t in range(HPI * NC) if not (t % NC == NC - 1 and t // NC in VHEADS)]
        for k, t in enumerate(order):
            qk(t)
            if k >= LAG:
                pv_reg(order[k - LAG])
        for k in range(len(pieces)):
            piece(k)
            if k < LAG:
                pv_reg(order[len(order) - LAG + k])
            if k in VDUE:
                j = VHEADS[VDUE.index(k)]
                pv(j, NC - 1, [vrows(j, True, g) for g in range(KC // KV)])
        outs = []
        for j in range(HPI):
            l = jnp.sum(jnp.concatenate(ls[j], axis=1), axis=0, keepdims=True)
            ok = jnp.minimum(ok, jnp.where((l >= L_LO) & (l <= L_HI), 1.0, 0.0))
            outs.append(accs[j] / l)
        oh_s[hh] = jnp.concatenate(outs, axis=0).T.astype(bf16)
        y_s[pl.ds(pl.multiple_of(hh * FR, FR), FR), :] = jnp.concatenate(y, axis=1)
        return ok

    ok = lax.fori_loop(0, NI, heads, jnp.ones((1, TQ), f32), unroll=2)

    @pl.when(i == 0)
    def _():
        w_cp[5].wait()

    @pl.when(i > 0)
    def _():
        for r in range(NO):
            o_cp(i - 1, r).wait()

    def finish():
        for r in range(NO):
            rows = pl.ds(pl.multiple_of(i * TQ + r * OR, OR), OR)
            o = jnp.concatenate([oh_s[g, r * OR:(r + 1) * OR, :] for g in range(NI)], axis=1)
            a = jnp.dot(o, wo_s[...], preferred_element_type=f32)
            out_s[r * OR:(r + 1) * OR, :] = (
                x_s[rows, :].astype(f32) + a + y_s[r * OR:(r + 1) * OR, :]).astype(out_s.dtype)
            o_cp(i, r).start()

    finish()

    @pl.when(jnp.min(ok) < 0.5)
    def _true_max_softmax():
        KB = 256

        def group(g, _):
            outs = []
            for j in range(HPI):
                q = qT_s[i * H + g * HPI + j, 0:DH, :]

                def chunk(c, carry, q=q):
                    m, l, acc = carry
                    ks = pl.ds(pl.multiple_of(c * KB, KB), KB)
                    s = jnp.dot(k_s[ks, 0:DH], q, preferred_element_type=f32)
                    m_new = jnp.maximum(m, jnp.max(s, axis=0, keepdims=True))
                    alpha = jnp.exp2(m - m_new)
                    p = jnp.exp2(s - m_new)
                    l = l * alpha + jnp.sum(p, axis=0, keepdims=True)
                    acc = acc * alpha + jnp.dot(vT_s[:, ks], p.astype(bf16), preferred_element_type=f32)
                    return m_new, l, acc

                _, l, acc = lax.fori_loop(0, S // KB, chunk, (
                    jnp.full((1, TQ), -jnp.inf, f32), jnp.zeros((1, TQ), f32), jnp.zeros((DH, TQ), f32)))
                outs.append(acc / l)
            oh_s[g] = jnp.concatenate(outs, axis=0).T.astype(bf16)
            return 0

        lax.fori_loop(0, NI, group, 0)
        for r in range(NO):
            o_cp(i, r).wait()
        finish()

    @pl.when(i == NT - 1)
    def _():
        for r in range(NO):
            o_cp(i, r).wait()


@jax.jit
def pallas_parallel_sum__grouped_kv_mqa__dense_activation_silu__prompt_kernel(
    A_x: jax.Array,
    A_wq: jax.Array,
    A_wk: jax.Array,
    A_wv: jax.Array,
    A_wo: jax.Array,
    B_x: jax.Array,
    B_w1: jax.Array,
    B_w2: jax.Array,
):
    del B_x
    out = pl.pallas_call(
        _kernel,
        grid=(NT,),
        in_specs=[pl.BlockSpec(memory_space=pl.ANY)] * 7,
        out_specs=pl.BlockSpec(memory_space=pl.ANY),
        out_shape=jax.ShapeDtypeStruct((S, D), A_x.dtype),
        scratch_shapes=[
            pltpu.VMEM((S, D), bf16),
            pltpu.VMEM((D, D), bf16),
            pltpu.VMEM((D, D), bf16),
            pltpu.VMEM((D, F), bf16),
            pltpu.VMEM((F, D), bf16),
            pltpu.SemaphoreType.DMA((NT + 6,)),
            pltpu.VMEM((S, D), bf16),
            pltpu.VMEM((D + 2 * DH, D), bf16),
            pltpu.VMEM((S, 128), bf16),
            pltpu.VMEM((DH, S), bf16),
            pltpu.VMEM((DH, NC * KV, 128), f32),
            pltpu.VMEM((DH, KC, 128), f32),
            pltpu.VMEM((DH, TQ), f32),
            pltpu.VMEM((NT * H, 2 * DH, TQ), bf16),
            pltpu.VMEM((NT * H, DH, TQ), f32),
            pltpu.VMEM((NT * NI, HPI, TQ), f32),
            pltpu.VMEM((NI, TQ, GW), bf16),
            pltpu.VMEM((TQ, D), f32),
            pltpu.VMEM((TQ, D), bf16),
            pltpu.SemaphoreType.DMA((NO,)),
        ],
        compiler_params=pltpu.CompilerParams(
            dimension_semantics=("arbitrary",), vmem_limit_bytes=100 * 2 ** 20),
    )(A_x.reshape(S, D), A_wq, A_wk.T, A_wv.T, A_wo, B_w1, B_w2)
    return out.reshape(A_x.shape)
```

```python
import functools

import jax
import jax.numpy as jnp
from jax import lax
import jax.experimental.pallas as pl
import jax.experimental.pallas.tpu as pltpu

S, D, H, DH, F = 2048, 512, 32, 16, 1792
LOG2E = 1.4426950408889634
EPS = 1e-5
NT_DIMS = (((1,), (1,)), ((), ()))
L_LO, L_HI = 2.0 ** -40, 2.0 ** 12
MARGIN = 1.0 + 2.0 ** -6

TQ, KC, UW, KV = 512, 128, 128, 16
KM = KC - KV
NC, NU, NT, NF = S // KC, TQ // UW, S // TQ, F // 128
HW = TQ // 2
LAG = 2
HPI = 16
NI = H // HPI
FR = TQ // NI
GW = HPI * DH
NO = 4
OR = TQ // NO
UPOS = (3, 6, 9, 12)
VHEADS = tuple(range(9, 16))
VBOUNDS = (1, 17, 32, 47, 61, 75, 89, 102)
VDUE = (6, 9, 13, 16, 20, 23, 26)

f32, bf16 = jnp.float32, jnp.bfloat16


def _ffn_pieces():
    w2p = [[('w2', (4 * g, 4 * g + 4, n, n + 1)) for n in range(4)] for g in range(3)]
    w2p.append([('w2', (12, 14, 0, 2)), ('w2', (12, 14, 2, 4))])
    w1p = [('w1', m) for m in range(NF)]
    pieces = w1p[0:5]
    for k in range(4):
        pieces += [w2p[0][k], w1p[5 + k]]
    for k in range(4):
        pieces += [w2p[1][k], w1p[9 + k]]
    return pieces + [w2p[2][0], w1p[13]] + w2p[2][1:] + w2p[3]


def _vunit_slots():
    out = {}
    for s, j in enumerate(VHEADS):
        slots = [divmod(q, FR // 8) for q in range(VBOUNDS[s] * FR // 32, VBOUNDS[s + 1] * FR // 32)]
        units = [(j, True, g, u) for g in range(KC // KV) for u in range(NU)]
        for k, un in enumerate(units):
            out[slots[((2 * k + 1) * len(slots)) // (2 * len(units))]] = un
    return out


def _kernel(x_hbm, wq_hbm, wkT_hbm, wvT_hbm, wo_hbm, w1_hbm, w2_hbm, o_hbm,
            x_s, wq_s, wo_s, w1_s, w2_s, sems,
            xn_s, wT_s, k_s, vT_s, kb_s, kb2_s, zero_s, qT_s, qf_s, sh_s, oh_s, y_s, out_s, oT_s, osems):
    i = pl.program_id(0)
    x_cp = [pltpu.make_async_copy(x_hbm.at[pl.ds(t * TQ, TQ)], x_s.at[pl.ds(t * TQ, TQ)], sems.at[t])
            for t in range(NT)]
    w_cp = [pltpu.make_async_copy(src, dst, sems.at[NT + n]) for n, (src, dst) in enumerate(
        [(wq_hbm, wq_s), (wkT_hbm, wT_s.at[pl.ds(0, DH)]), (wvT_hbm, wT_s.at[pl.ds(DH, DH)]),
         (w1_hbm, w1_s), (w2_hbm, w2_s), (wo_hbm, wo_s)])]

    def o_cp(t, r):
        return pltpu.make_async_copy(out_s.at[pl.ds(r * OR, OR)],
                                     o_hbm.at[pl.ds(pl.multiple_of(t * TQ + r * OR, OR), OR)], osems.at[r])

    @pl.when(i == 0)
    def _prologue():
        x_cp[0].start()
        for cp in w_cp[:3] + x_cp[1:] + w_cp[3:]:
            cp.start()
        zero_s[...] = jnp.zeros(zero_s.shape, f32)
        hrow = lax.broadcasted_iota(jnp.int32, (H, D), 0)
        hcol = lax.broadcasted_iota(jnp.int32, (H, D), 1)
        blockdiag = jnp.where(hcol // DH == hrow, 1.0, 0.0).astype(bf16)
        kn2s, nqns = {}, {}

        def ln(t):
            rows = pl.ds(t * TQ, TQ)
            x = x_s[rows, :].astype(f32)
            xc = x - jnp.mean(x, axis=-1, keepdims=True)
            v = jnp.mean(xc * xc, axis=-1, keepdims=True)
            xn_s[rows, :] = (xc * lax.rsqrt(v + EPS)).astype(bf16)

        def proj(z):
            t, c0 = divmod(z * HW, TQ)
            res = lax.dot_general(wT_s[...], xn_s[z * HW:(z + 1) * HW, :], NT_DIMS,
                                  preferred_element_type=f32)
            vT_s[:, z * HW:(z + 1) * HW] = res[DH:2 * DH].astype(bf16)
            kT = res[0:DH].astype(bf16).astype(f32)
            kfull = jnp.concatenate([kT, jnp.zeros((128 - DH, HW), f32)], axis=0).T
            nk = HW // KC
            kv_rows = kfull.reshape(nk, KC, 128)[:, KM:, :].reshape(nk * KV, 128)
            for d in range(DH):
                kb_s[d, z * nk * KV:(z + 1) * nk * KV, :] = jnp.broadcast_to(kv_rows[:, d:d + 1], (nk * KV, 128))
            if z == 2 * NT - 1:
                for d in range(DH):
                    kb2_s[d] = jnp.broadcast_to(kfull[HW - KC:, d:d + 1], (KC, 128))
            kn2s[z] = jnp.sum(kT * kT, axis=0, keepdims=True)
            k_s[z * HW:(z + 1) * HW, :] = kfull.astype(bf16)
            qb = (res[2 * DH:] * (DH ** -0.5 * LOG2E)).astype(bf16)
            qT_s[t * H:(t + 1) * H, 0:DH, c0:c0 + HW] = qb.reshape(H, DH, HW)
            qf_s[t * H:(t + 1) * H, :, c0:c0 + HW] = qb.astype(f32).reshape(H, DH, HW)

        def norm(z):
            t, c0 = divmod(z * HW, TQ)
            qf = qf_s[t * H:(t + 1) * H, :, c0:c0 + HW].reshape(D, HW)
            qn2 = jnp.dot(blockdiag, (qf * qf).astype(bf16), preferred_element_type=f32)
            nqn = (jnp.sqrt(qn2) * -MARGIN).astype(bf16).astype(f32)
            row0 = lax.broadcasted_iota(jnp.int32, (DH, HW), 0) == 0
            for h in range(H):
                qT_s[t * H + h, DH:, c0:c0 + HW] = jnp.where(
                    row0, jnp.broadcast_to(nqn[h:h + 1], (DH, HW)), 0.0).astype(bf16)
            nqns[z] = nqn

        x_cp[0].wait()
        ln(0)
        for cp in w_cp[:3]:
            cp.wait()
        wT_s[2 * DH:, :] = wq_s[...].astype(f32).T.astype(bf16)
        proj(0)
        x_cp[1].wait()
        proj(1); ln(1); norm(0); proj(2)
        x_cp[2].wait()
        x_cp[3].wait()
        proj(3); ln(2); norm(1); ln(3); proj(4); norm(2); proj(5); norm(3); proj(6); norm(4); norm(5)
        proj(7); norm(6); norm(7)
        kn2 = functools.reduce(jnp.maximum, [kn2s[z] for z in range(2 * NT)])
        kmax = (jnp.sqrt(jnp.max(kn2, axis=1, keepdims=True)) * MARGIN).astype(bf16).astype(f32)
        k_s[:, DH:DH + 1] = jnp.broadcast_to(kmax, (S, 1)).astype(bf16)
        for z in range(2 * NT):
            t, c0 = divmod(z * HW, TQ)
            sh_s[t * NI:(t + 1) * NI, :, c0:c0 + HW] = (nqns[z] * kmax).reshape(NI, HPI, HW)
        for cp in w_cp[3:5]:
            cp.wait()

    pieces, vslots = _ffn_pieces(), _vunit_slots()

    def heads(hh, ok):
        hidx = [i * H + hh * HPI + j for j in range(HPI)]
        frows = pl.ds(pl.multiple_of(i * TQ + hh * FR, FR), FR)
        sidx = i * NI + hh
        accs = [zero_s[...] for _ in range(HPI)]
        ls = [[jnp.zeros((8, UW), f32) for _ in range(NU)] for _ in range(HPI)]
        always = zero_s[0:8, 0:UW] == 0.0
        ps, pvs, hact = {}, {}, {}
        y = [None] * (D // 128)

        @functools.cache
        def q_rows(j, u):
            cols = slice(u * UW, (u + 1) * UW)
            return ([jnp.broadcast_to(qf_s[hidx[j], d:d + 1, cols], (KV, UW)) for d in range(DH)],
                    jnp.broadcast_to(sh_s[sidx, j:j + 1, cols], (KV, UW)))

        @functools.cache
        def k_rows(last, g):
            ref = kb2_s if last else kb_s
            return [ref[d, g * KV:(g + 1) * KV, :] for d in range(DH)]

        def unit(j, last, g, u, anchor=None):
            if anchor is not None:
                ls[j][u] = jnp.where(always, ls[j][u], anchor)
            q, sv = q_rows(j, u)
            k = k_rows(last, g)
            for d in range(DH):
                sv = sv + k[d] * q[d]
            p = jnp.exp2(sv)
            ls[j][u] = ls[j][u] + p[0:8] + p[8:16]
            pvs[(j, last, g, u)] = p

        def vrows(j, last, g):
            return jnp.concatenate([pvs.pop((j, last, g, u)) for u in range(NU)], axis=1)

        def qk(t):
            j, c = divmod(t, NC)
            p = jnp.exp2(jnp.dot(k_s[c * KC:c * KC + KM, 0:2 * DH], qT_s[hidx[j]], preferred_element_type=f32))
            l = jnp.concatenate(ls[j], axis=1)
            for r in range(KM // 8):
                l = l + p[r * 8:(r + 1) * 8]
                if r in UPOS:
                    u = UPOS.index(r)
                    ls[j][u] = l[:, u * UW:(u + 1) * UW]
                    unit(j, False, c, u)
                    l = jnp.concatenate(([l[:, :u * UW]] if u else []) + [ls[j][u]] +
                                        ([l[:, (u + 1) * UW:]] if u < NU - 1 else []), axis=1)
            ls[j] = [l[:, u * UW:(u + 1) * UW] for u in range(NU)]
            ps[t] = p

        def pv(j, c, parts):
            p = jnp.concatenate(parts, axis=0).astype(bf16)
            accs[j] = accs[j] + jnp.dot(vT_s[:, c * KC:(c + 1) * KC], p, preferred_element_type=f32)

        def pv_reg(t):
            j, c = divmod(t, NC)
            pv(j, c, [ps.pop(t), vrows(j, False, c)])

        def piece(k):
            kind, a = pieces[k]
            if kind == 'w1':
                res = jnp.dot(xn_s[frows, :], w1_s[:, a * 128:(a + 1) * 128], preferred_element_type=f32)
            else:
                k0, k1, n0, n1 = a
                res = jnp.dot(jnp.concatenate([hact[kk] for kk in range(k0, k1)], axis=1),
                              w2_s[k0 * 128:k1 * 128, n0 * 128:n1 * 128], preferred_element_type=f32)
            for r in range(FR // 8):
                if (k, r) in vslots:
                    unit(*vslots[(k, r)], anchor=res[r * 8:(r + 1) * 8, 0:UW])
            if kind == 'w1':
                hm = 0.5 * res
                hact[a] = (hm + hm * jnp.tanh(hm)).astype(bf16)
            else:
                for n in range(n0, n1):
                    pn = res[:, (n - n0) * 128:(n - n0 + 1) * 128]
                    y[n] = pn if y[n] is None else y[n] + pn

        order = [t for t in range(HPI * NC) if not (t % NC == NC - 1 and t // NC in VHEADS)]
        for k, t in enumerate(order):
            qk(t)
            if k >= LAG:
                pv_reg(order[k - LAG])
        for k in range(len(pieces)):
            piece(k)
            if k < LAG:
                pv_reg(order[len(order) - LAG + k])
            if k in VDUE:
                j = VHEADS[VDUE.index(k)]
                pv(j, NC - 1, [vrows(j, True, g) for g in range(KC // KV)])
        outs = []
        for j in range(HPI):
            l = jnp.sum(jnp.concatenate(ls[j], axis=1), axis=0, keepdims=True)
            ok = jnp.minimum(ok, jnp.where((l >= L_LO) & (l <= L_HI), 1.0, 0.0))
            outs.append(accs[j] / l)
        oh_s[hh] = jnp.concatenate(outs, axis=0).T.astype(bf16)
        y_s[pl.ds(pl.multiple_of(hh * FR, FR), FR), :] = jnp.concatenate(y, axis=1)
        return ok

    ok = lax.fori_loop(0, NI, heads, jnp.ones((1, TQ), f32))

    @pl.when(i == 0)
    def _():
        w_cp[5].wait()

    @pl.when(i > 0)
    def _():
        for r in range(NO):
            o_cp(i - 1, r).wait()

    def finish():
        for r in range(NO):
            rows = pl.ds(pl.multiple_of(i * TQ + r * OR, OR), OR)
            o = jnp.concatenate([oh_s[g, r * OR:(r + 1) * OR, :] for g in range(NI)], axis=1)
            a = jnp.dot(o, wo_s[...], preferred_element_type=f32)
            out_s[r * OR:(r + 1) * OR, :] = (
                x_s[rows, :].astype(f32) + a + y_s[r * OR:(r + 1) * OR, :]).astype(out_s.dtype)
            o_cp(i, r).start()

    finish()

    @pl.when(jnp.min(ok) < 0.5)
    def _true_max_softmax():
        KB = 256

        def head(h, _):
            q = qT_s[i * H + h, 0:DH, :]

            def chunk(c, carry):
                m, l, acc = carry
                ks = pl.ds(pl.multiple_of(c * KB, KB), KB)
                s = jnp.dot(k_s[ks, 0:DH], q, preferred_element_type=f32)
                m_new = jnp.maximum(m, jnp.max(s, axis=0, keepdims=True))
                alpha = jnp.exp2(m - m_new)
                p = jnp.exp2(s - m_new)
                l = l * alpha + jnp.sum(p, axis=0, keepdims=True)
                acc = acc * alpha + jnp.dot(vT_s[:, ks], p.astype(bf16), preferred_element_type=f32)
                return m_new, l, acc

            _, l, acc = lax.fori_loop(0, S // KB, chunk, (
                jnp.full((1, TQ), -jnp.inf, f32), jnp.zeros((1, TQ), f32), jnp.zeros((DH, TQ), f32)))
            oT_s[pl.ds(pl.multiple_of(h * DH, DH), DH), :] = acc / l
            return 0

        lax.fori_loop(0, H, head, 0)
        for g in range(NI):
            oh_s[g] = oT_s[g * GW:(g + 1) * GW, :].T.astype(bf16)
        for r in range(NO):
            o_cp(i, r).wait()
        finish()

    @pl.when(i == NT - 1)
    def _():
        for r in range(NO):
            o_cp(i, r).wait()


@jax.jit
def pallas_parallel_sum__grouped_kv_mqa__dense_activation_silu__prompt_kernel(
    A_x: jax.Array,
    A_wq: jax.Array,
    A_wk: jax.Array,
    A_wv: jax.Array,
    A_wo: jax.Array,
    B_x: jax.Array,
    B_w1: jax.Array,
    B_w2: jax.Array,
):
    del B_x
    out = pl.pallas_call(
        _kernel,
        grid=(NT,),
        in_specs=[pl.BlockSpec(memory_space=pl.ANY)] * 7,
        out_specs=pl.BlockSpec(memory_space=pl.ANY),
        out_shape=jax.ShapeDtypeStruct((S, D), A_x.dtype),
        scratch_shapes=[
            pltpu.VMEM((S, D), bf16),
            pltpu.VMEM((D, D), bf16),
            pltpu.VMEM((D, D), bf16),
            pltpu.VMEM((D, F), bf16),
            pltpu.VMEM((F, D), bf16),
            pltpu.SemaphoreType.DMA((NT + 6,)),
            pltpu.VMEM((S, D), bf16),
            pltpu.VMEM((D + 2 * DH, D), bf16),
            pltpu.VMEM((S, 128), bf16),
            pltpu.VMEM((DH, S), bf16),
            pltpu.VMEM((DH, NC * KV, 128), f32),
            pltpu.VMEM((DH, KC, 128), f32),
            pltpu.VMEM((DH, TQ), f32),
            pltpu.VMEM((NT * H, 2 * DH, TQ), bf16),
            pltpu.VMEM((NT * H, DH, TQ), f32),
            pltpu.VMEM((NT * NI, HPI, TQ), f32),
            pltpu.VMEM((NI, TQ, GW), bf16),
            pltpu.VMEM((TQ, D), f32),
            pltpu.VMEM((TQ, D), bf16),
            pltpu.VMEM((D, TQ), f32),
            pltpu.SemaphoreType.DMA((NO,)),
        ],
        compiler_params=pltpu.CompilerParams(
            dimension_semantics=("arbitrary",), vmem_limit_bytes=100 * 2 ** 20),
    )(A_x.reshape(S, D), A_wq, A_wk.T, A_wv.T, A_wo, B_w1, B_w2)
    return out.reshape(A_x.shape)
```
